```python
import jax
import jax.numpy as jnp

def _softmax(x, axis=-1):
    return jax.nn.softmax(x, axis=axis)
def _gelu(x):
    return jax.nn.gelu(x, approximate=True)
def _silu(x):
    return jax.nn.silu(x)
def _sigmoid(x):
    return jax.nn.sigmoid(x)
def _layernorm(x, axis=-1, eps=1e-5):
    m = jnp.mean(x, axis=axis, keepdims=True)
    v = jnp.var(x, axis=axis, keepdims=True)
    return (x - m) / jnp.sqrt(v + eps)
def _scatter_add(tgt, idx, src, axis=0):
    return tgt.at[idx].add(src)
def _segment_sum(src, seg, n):
    return jax.ops.segment_sum(src, seg, n)
class _Rng:
    def __init__(self, key):
        self._k = key
    def _next(self):
        self._k, sub = jax.random.split(self._k)
        return sub
    def normal(self, shape):
        return jax.random.normal(self._next(), shape, dtype=jnp.bfloat16)
    def randint(self, lo, hi, shape):
        return jax.random.randint(self._next(), shape, lo, hi, dtype=jnp.int32)
    def uniform(self, shape, lo=0.0, hi=1.0):
        return jax.random.uniform(self._next(), shape, jnp.bfloat16, lo, hi)
    def permutation(self, n):
        return jax.random.permutation(self._next(), n)


kernel_name = 'recurrent_scan__compressed_kv_cla__dense_activation_gelu__decode'

def setup_inputs():
    _rng = _Rng(jax.random.key(int.from_bytes(__import__("os").urandom(4), "little")))
    _w = (lambda a: (lambda t: t.astype(jnp.bfloat16) if jnp.issubdtype(t.dtype, jnp.floating) else t)(jnp.asarray(a)))
    def _A_setup():
        B, H, Sq, Sk, D, M = 2, 32, 1, 16384, 128, 512
        Dc = 4 * D
        return {
            "x": _w((lambda *s: _rng.normal(s) * 0.05)(B, Sq, M)),
            "c_kv": _w((lambda *s: _rng.normal(s) * 0.05)(B, Sk, Dc)),
            "w_q": _w((lambda *s: _rng.normal(s) * 0.05)(M, H, D) * (M ** -0.5)),
            "w_uk": _w((lambda *s: _rng.normal(s) * 0.05)(Dc, H, D) * (Dc ** -0.5)),
            "w_uv": _w((lambda *s: _rng.normal(s) * 0.05)(Dc, H, D) * (Dc ** -0.5)),
            "w_o": _w((lambda *s: _rng.normal(s) * 0.05)(H, D, M) * ((H * D) ** -0.5)),
        }
    _A_in = _A_setup()

    def _B_setup():
        B, S, D, F = 2, 1, 512, 1792
        return {
            "x": _w((lambda *s: _rng.normal(s) * 0.05)(B, S, D)),
            "w1": _w((lambda *s: _rng.normal(s) * 0.05)(D, F) * (D ** -0.5)),
            "b1": _w((lambda *s: _rng.normal(s) * 0.05)(F) * 0.01),
            "w2": _w((lambda *s: _rng.normal(s) * 0.05)(F, D) * (F ** -0.5)),
            "b2": _w((lambda *s: _rng.normal(s) * 0.05)(D) * 0.01),
        }
    _B_in = _B_setup()

    return {
        "A_x": _A_in["x"],
        "A_c_kv": _A_in["c_kv"],
        "A_w_q": _A_in["w_q"],
        "A_w_uk": _A_in["w_uk"],
        "A_w_uv": _A_in["w_uv"],
        "A_w_o": _A_in["w_o"],
        "B_x": _B_in["x"],
        "B_w1": _B_in["w1"],
        "B_b1": _B_in["b1"],
        "B_w2": _B_in["w2"],
        "B_b2": _B_in["b2"],
    }

def reference(A_x, A_c_kv, A_w_q, A_w_uk, A_w_uv, A_w_o, B_x, B_w1, B_b1, B_w2, B_b2):
    def _A_ref(x, c_kv, w_q, w_uk, w_uv, w_o):
        B, Sq, M = x.shape[0], x.shape[1], x.shape[2]
        Sk = c_kv.shape[1]
        H, D = w_q.shape[1], w_q.shape[2]
        q = jnp.einsum("bqm,mhd->bhqd", x, w_q)
        k = jnp.einsum("bkc,chd->bhkd", c_kv, w_uk)
        v = jnp.einsum("bkc,chd->bhkd", c_kv, w_uv)
        scores = jnp.einsum("bhqd,bhkd->bhqk", q, k) * (D ** -0.5)
        off = Sk - Sq
        qi = jnp.arange(Sq)[:, None]
        kj = jnp.arange(Sk)[None, :]
        cmask = kj <= (qi + off)
        scores = jnp.where(cmask[None, None], scores, -1e9)
        p = _softmax(scores, axis=-1)
        ctx = jnp.einsum("bhqk,bhkd->bhqd", p, v)
        return jnp.einsum("bhqd,hdm->bqm", ctx, w_o)

    def _B_ref(x, w1, b1, w2, b2):
        h = jnp.einsum("bsd,df->bsf", x, w1) + b1
        h = _gelu(h)
        return jnp.einsum("bsf,fd->bsd", h, w2) + b2

    x = A_x
    xn = _layernorm(x, axis=-1)
    s = _A_ref(xn, A_c_kv, A_w_q, A_w_uk, A_w_uv, A_w_o)
    g = _silu(_B_ref(xn, B_w1, B_b1, B_w2, B_b2))
    return x + s * g
```

```python
import jax
import jax.numpy as jnp
from jax import lax
import jax.experimental.pallas as pl
import jax.experimental.pallas.tpu as pltpu
import contextlib

F32 = jnp.float32
BF16 = jnp.bfloat16
B, H, SK, D, M, DC, F = 2, 32, 16384, 128, 512, 512, 1792
LOG2E = 1.4426950408889634
NT = (((1,), (1,)), ((), ()))


def _loop(lo, hi, body):
    lax.fori_loop(lo, hi, lambda i, _: body(i), None)


def _rows8(v):
    return jnp.concatenate([v[:, j * 128:(j + 1) * 128] for j in range(M // 128)], axis=0)


def make(TR=False, LAG=26, N0=1, OCUTS=(0, 4, 8, 12, 14, 16), TCUTS=(0, 64, 128, 192, 224, 248, 256), TMXU=0, OVPU=0,
         FG=4, AHEAD=16, POST=205, NOCOMP=False):
    W_VIEW = (4, 128, H, D)
    C_VIEW = (B * 16, SK // 16, DC)
    O_VIEW = (4, 8 * D, M)
    F_VIEW = (112 * 8, 8, 128) if FG == 4 else (2, 56 * 8, 8, 128)
    G_VIEW = (F, M) if FG == 4 else (2, F // 2, M)
    R_C, R_O, R_END = 64, 192, 208
    TAIL = TCUTS[-1]
    T0 = 8 * D - TAIL
    BK = 2048

    def scope(name):
        return jax.named_scope('@' + name) if TR else contextlib.nullcontext()

    def kernel(x_hbm, c_hbm, wq_hbm, wk_hbm, wv_hbm, wo_hbm, w1_hbm, b1_hbm, w2_hbm, b2_hbm, o_hbm,
               c_buf, wq_buf, wk_buf, wv_buf, wo_buf, w1_buf, w2_buf,
               flat, qa_ref, ctx_ref, lhs_ref, mul_ref, o_buf, x_buf, b1_buf, b2_buf,
               sem_w, sem_c, sem_o, sem_t, sem_small):
        def fetch(hbm, buf, idx, sem, queue):
            pltpu.make_async_copy(hbm.at[idx], buf.at[idx], sem).start(priority=queue)

        def wait_filled(buf, sem, name='w'):
            with scope(name):
                pltpu.make_async_copy(buf, buf, sem).wait()

        def rows(start, n, align=16):
            return pl.ds(start if isinstance(start, int) else pl.multiple_of(start, align), n)

        def runs(first, queue, n=4):
            return pl.ds(first, N0) if queue == 0 else pl.ds(first + N0, n - N0)

        def step(at, r, t, queue):
            if at < R_C:
                if t < 3:
                    hbm, buf = ((wq_hbm, wq_buf), (wk_hbm, wk_buf), (wv_hbm, wv_buf))[t]
                    fetch(hbm, buf, (runs(0, queue), pl.ds(r * 2, 2)), sem_w.at[t], queue)
                elif queue == 0:
                    fetch(w1_hbm, w1_buf, pl.ds(r * 8, 8), sem_w.at[3], 0)
                    if at < 48:
                        fetch(w1_hbm, w1_buf, pl.ds(r * 8 + 512, 8), sem_w.at[3], 0)
                        fetch(w2_hbm, w2_buf, rows(r * 16, 16), sem_w.at[4], 0)
                else:
                    fetch(w2_hbm, w2_buf, rows(r * 16 + (1024 if at < 48 else 0), 16), sem_w.at[4], 1)
            elif at < R_O:
                u = r - R_C
                fetch(c_hbm, c_buf, (runs((u >> 6) * 16 + t * 4, queue), rows((u & 63) * 16, 16)), sem_c.at[u >> 3], queue)
            elif at < R_END:
                off = (t % 2) * 512 + (t // 2) * 16
                group = sum(at - R_O + (t // 2) / 2 >= c for c in OCUTS[1:])
                n = 4 if (at - R_O) * 32 + off < T0 else 3
                fetch(wo_hbm, wo_buf, (runs(0, queue, n), rows((r - R_O) * 32 + off, 16)), sem_o.at[group], queue)
            else:
                s = (at - R_END) * 4 + t
                big = (TAIL - 128) // 64
                if s < big:
                    row, idx = s * 64 + queue * 32, (32, pl.ds(0, M))
                elif queue == 1 and s < big + 32:
                    row, idx = big * 64 + (s - big) // 2 * 8, (8, pl.ds((s - big) % 2 * 256, 256))
                else:
                    return
                fetch(wo_hbm, wo_buf, (3, pl.ds(T0 + row, idx[0]), idx[1]), sem_t.at[sum(row >= c for c in TCUTS[1:])], queue)

        def issue_round(at, r):
            for t in range(4):
                step(at, r, t, 0)
                step(at + (t + LAG) // 4, r + (t + LAG) // 4, (t + LAG) % 4, 1)

        edges = [48, R_C, R_O + (T0 - 512) // 32] + [R_O + int(c + d) for c in OCUTS for d in (0, 0.5)] + list(range(R_END, R_END + 10))
        edges = sorted({e - d for e in edges for d in (0, LAG // 4, (LAG + 3) // 4)})

        def issue(lo, hi):
            cuts = [lo] + [e for e in edges if lo < e < hi] + [hi]
            with scope(f'i{hi}'):
                for a, b in zip(cuts, cuts[1:]):
                    if b == a + 1:
                        issue_round(a, a)
                    else:
                        _loop(a, b, lambda r: issue_round(a, r))

        def issue_c(lo, hi):
            with scope('ic'):
                _loop(lo, hi, lambda r: issue_round(R_C, r))

        x_copy = pltpu.make_async_copy(x_hbm, x_buf, sem_small.at[0])
        b1_copy = pltpu.make_async_copy(b1_hbm, b1_buf, sem_small.at[1])
        b2_copy = pltpu.make_async_copy(b2_hbm, b2_buf, sem_small.at[2])

        step(0, 0, 0, 0)
        for s in range(LAG + 1):
            step(s // 4, s // 4, s % 4, 1)
        for t in range(1, 4):
            step(0, 0, t, 0)
            step((t + LAG) // 4, (t + LAG) // 4, (t + LAG) % 4, 1)
        issue(1, 4)
        for c in (x_copy, b1_copy, b2_copy):
            c.start()
        if NOCOMP:
            issue(4, R_END + 3)
            for c in (x_copy, b1_copy, b2_copy):
                c.wait()
            for i, v in enumerate((wq_buf, wk_buf, wv_buf, w1_buf, w2_buf)):
                wait_filled(v, sem_w.at[i])
            for i in range(16):
                wait_filled(c_buf.at[pl.ds(0, 16), pl.ds(0, 128)], sem_c.at[i])
            o_buf[...] = jnp.zeros((8, 128), BF16)
            for g, (lo, hi) in enumerate(zip(OCUTS, OCUTS[1:])):
                wait_filled(wo_buf.at[:, pl.ds(lo * 32, (hi - lo) * 32)], sem_o.at[g])
                wait_filled(wo_buf.at[pl.ds(0, 4 if 512 + lo * 32 < T0 else 3), pl.ds(lo * 32, (hi - lo) * 32)], sem_o.at[g])
            for g, (lo, hi) in enumerate(zip(TCUTS, TCUTS[1:])):
                wait_filled(wo_buf.at[3, pl.ds(T0 + lo, hi - lo)], sem_t.at[g])
            o_copy = pltpu.make_async_copy(o_buf, o_hbm, sem_small.at[0])
            o_copy.start()
            o_copy.wait()
            return
        issue(4, 73)

        x_copy.wait()
        x = x_buf[...].astype(F32)
        xc = x - jnp.mean(x, axis=-1, keepdims=True)
        var = jnp.mean(xc * xc, axis=-1, keepdims=True)
        xn = (xc * lax.rsqrt(var + 1e-5)).astype(BF16)

        def iota(shape, axis):
            return lax.broadcasted_iota(jnp.int32, shape, axis)

        def same_head():
            return iota((H, 128), 1) % H == iota((H, 128), 0)

        def same_quad():
            return (iota((128, DC), 1) // 4 == iota((128, DC), 0)).astype(F32).astype(BF16)

        def contract_rows(v, w_buf):
            v4 = jnp.concatenate([jnp.where(iota((H, DC), 1) % 4 == j, v, 0.0) for j in range(4)], axis=0)
            flat[...] = lax.dot_general(same_quad(), v4.astype(BF16), NT, preferred_element_type=F32)
            lhs = jnp.concatenate([jnp.where(same_head(), flat[t:t + 1, :], 0.0).astype(BF16) for t in range(128)], axis=1)
            return jnp.dot(lhs, w_buf[...].reshape(DC * H, D), preferred_element_type=F32)

        def contract_lanes(v, w_buf, scale, before_half):
            def half(k):
                before_half(k)
                w = w_buf[pl.ds(2 * k, 2)].reshape(DC * H // 2, D)
                r = lax.dot_general(v.astype(BF16), w, NT, preferred_element_type=F32)
                for t in range(64):
                    flat[pl.ds(k * 64 + t, 1), :] = jnp.sum(jnp.where(same_head(), r[:, t * 128:(t + 1) * 128], 0.0), axis=0, keepdims=True)
            _loop(0, 2, half)
            v4 = jnp.dot((flat[...] * scale).T.astype(BF16), same_quad(), preferred_element_type=F32)
            out = v4[:H]
            for j in range(1, 4):
                out = jnp.where(iota((H, DC), 1) % 4 == j, v4[j * H:(j + 1) * H], out)
            return out.astype(BF16)

        wait_filled(wq_buf, sem_w.at[0], 'wq')
        wait_filled(wk_buf, sem_w.at[1], 'wk')
        wait_filled(wv_buf, sem_w.at[2], 'wv')

        def absorb(b):
            xb = jnp.where(b == 0, xn[0:1].astype(F32), xn[1:2].astype(F32))
            q = contract_rows(jnp.broadcast_to(xb, (H, M)), wq_buf)
            qa_ref[b] = contract_lanes(q, wk_buf, D ** -0.5 * LOG2E, lambda k: issue_c(73 + 12 * b + 4 * k, 77 + 12 * b + 4 * k))
            issue_c(81 + 12 * b, 85 + 12 * b)

        _loop(0, B, absorb)

        wait_filled(w1_buf, sem_w.at[3])
        wait_filled(w2_buf, sem_w.at[4])
        b1_copy.wait()
        b2_copy.wait()
        w1 = w1_buf[...].reshape(M // 8, F // 128, 8, 128)
        w1 = jnp.concatenate([w1[:, j].reshape(M, 128) for j in range(F // 128)], axis=1)
        hid = jnp.dot(xn, w1, preferred_element_type=F32)
        hid = jax.nn.gelu(hid + b1_buf[...].astype(F32).reshape(1, F), approximate=True).astype(BF16)
        issue_c(97, 99)
        z = jnp.dot(hid, w2_buf[...].reshape(F, M), preferred_element_type=F32)
        z8 = _rows8(z + b2_buf[...].astype(F32).reshape(1, M))
        g8 = z8 * jax.nn.sigmoid(z8)
        x8 = _rows8(x)

        last_c = R_O - (LAG + 3) // 4

        def issued(i):
            return jnp.minimum(jnp.maximum(104 + 5 * i + jnp.where(i >= 8, 4, 0), R_C + AHEAD + 8 * i), last_c)

        def block(b, g, carry):
            m_prev, l_prev, acc = carry
            i = b * 8 + g
            issue_c(issued(i - 1) + jnp.where(i == 8, 5, 0), issued(i))
            for k in (14, 15):
                pl.when(i == k)(lambda: issue(max(last_c, R_C + AHEAD + 8 * (k - 1)), R_C + AHEAD + 8 * k))
            part = (pl.ds(b * 16, 16), rows(g * 128, 128, 128))
            wait_filled(c_buf.at[part], sem_c.at[i], 'c')
            c = c_buf[part].reshape(BK, DC)
            sc = lax.dot_general(qa_ref[b], c, NT, preferred_element_type=F32)
            m_new = jnp.maximum(m_prev, jnp.max(sc, axis=1, keepdims=True))
            p = jnp.exp2(sc - m_new)
            alpha = jnp.exp2(m_prev - m_new)
            pv = jnp.dot(p.astype(BF16), c, preferred_element_type=F32)
            return m_new, alpha * l_prev + jnp.sum(p, axis=1, keepdims=True), alpha * acc + pv

        def attend(b):
            init = (jnp.full((H, 1), -jnp.inf, F32), jnp.zeros((H, 1), F32), jnp.zeros((H, DC), F32))
            _, l, acc = lax.fori_loop(0, SK // BK, lambda g, carry: block(b, g, carry), init)
            pl.when(b == 0)(lambda: issue_c(issued(7), issued(7) + 5))
            pl.when(b == 1)(lambda: issue(R_C + AHEAD + 120, POST))
            ctx_ref[b] = contract_rows(acc / l, wv_buf)

        _loop(0, B, attend)
        issue(POST, R_END + 3)
        groups = []
        for g, (lo, hi) in enumerate(zip(OCUTS, OCUTS[1:])):
            r, n = int(lo * 32), int((hi - lo) * 32)
            n1 = 4 if 512 + r < T0 else 3
            groups.append(([(wo_buf.at[:, pl.ds(r, n)], sem_o.at[g]), (wo_buf.at[pl.ds(0, n1), pl.ds(512 + r, n)], sem_o.at[g])],
                           [(a, r, n) for a in range(4)] + [(a, 512 + r, n) for a in range(n1)], g < len(OCUTS) - 1 - OVPU))
        for g, (lo, hi) in enumerate(zip(TCUTS, TCUTS[1:])):
            groups.append(([(wo_buf.at[3, pl.ds(T0 + lo, hi - lo)], sem_t.at[g])], [(3, T0 + lo, hi - lo)], g < TMXU))

        def gather(parts):
            return jnp.concatenate([ctx_ref[:, a * 8 + r // D, :][:, r % D:r % D + n] for a, r, n in parts], axis=1)

        for g, (_, parts, mxu) in enumerate(groups):
            if mxu:
                lhs_ref[g, :B, :sum(n for _, _, n in parts)] = gather(parts)
        vpu = [p for _, parts, mxu in groups if not mxu for p in parts]
        nv = sum(n for _, _, n in vpu)
        pad = -nv % 128
        cb = gather(([(0, 0, pad)] if pad else []) + vpu).astype(BF16).astype(F32)
        for b in range(B):
            for k in range(0, nv + pad, 128):
                mul_ref[b, k:k + 128] = jnp.broadcast_to(cb[b:b + 1, k:k + 128], (128, 128)).T

        s = jnp.zeros((B, M), F32)
        part = [[None] * (M // 128) for _ in range(B)]
        at = pad
        for g, (waits, parts, mxu) in enumerate(groups):
            for v, sem in waits:
                wait_filled(v, sem, 'o' if mxu else 't')
            if mxu:
                rhs = jnp.concatenate([wo_buf[a, r:r + n] for a, r, n in parts], axis=0)
                s = s + jnp.dot(lhs_ref[g, :B, :rhs.shape[0]].astype(BF16), rhs, preferred_element_type=F32)
                continue
            for a, r0, n in parts:
                for r in range(r0, r0 + n, 8):
                    w = wo_buf[a, r:r + 8].astype(F32)
                    for b in range(B):
                        mul = mul_ref[b, at:at + 8, :]
                        for j in range(M // 128):
                            t = w[:, j * 128:(j + 1) * 128] * mul
                            part[b][j] = t if part[b][j] is None else part[b][j] + t
                    at += 8
        base8 = x8 + _rows8(s) * g8

        sl = lax.broadcasted_iota(jnp.int32, (8, 128), 0)

        def merge(lo, hi, k):
            m = (sl & k) != 0
            if k == 4:
                return jnp.where(m, hi, lo) + pltpu.roll(jnp.where(m, lo, hi), 4, 0)
            return jnp.where(m, hi, lo) + jnp.where(m, pltpu.roll(hi, k, 0), pltpu.roll(lo, 8 - k, 0))

        r4 = [[merge(part[b][j], part[b][j + 2], 4) for j in range(2)] for b in range(B)]
        r2 = [merge(r4[b][0], r4[b][1], 2) for b in range(B)]
        o_buf[...] = (base8 + g8 * merge(r2[0], r2[1], 1)).astype(BF16)
        o_copy = pltpu.make_async_copy(o_buf, o_hbm, sem_small.at[0])
        o_copy.start()
        o_copy.wait()

    def fn(A_x, A_c_kv, A_w_q, A_w_uk, A_w_uv, A_w_o, B_x, B_w1, B_b1, B_w2, B_b2):
        hbm = pl.BlockSpec(memory_space=pltpu.HBM)
        dma_sems = pltpu.SemaphoreType.DMA
        w1 = B_w1.reshape(M // 8, 8, F // 128, 128).transpose(0, 2, 1, 3).reshape(F_VIEW)
        out = pl.pallas_call(
            kernel,
            out_shape=jax.ShapeDtypeStruct((8, 128), BF16),
            in_specs=[hbm] * 10,
            out_specs=hbm,
            scratch_shapes=[
                pltpu.VMEM(C_VIEW, BF16), pltpu.VMEM(W_VIEW, BF16), pltpu.VMEM(W_VIEW, BF16),
                pltpu.VMEM(W_VIEW, BF16), pltpu.VMEM(O_VIEW, BF16),
                pltpu.VMEM(F_VIEW, BF16), pltpu.VMEM(G_VIEW, BF16),
                pltpu.VMEM((128, 128), F32), pltpu.VMEM((B, H, DC), BF16), pltpu.VMEM((B, H, D), F32),
                pltpu.VMEM((16, 8, 1024), F32), pltpu.VMEM((B, 8 * D, 128), F32), pltpu.VMEM((8, 128), BF16),
                pltpu.VMEM((B, M), BF16), pltpu.VMEM((F,), BF16), pltpu.VMEM((M,), BF16),
                dma_sems((5,)), dma_sems((16,)), dma_sems((len(OCUTS) - 1,)), dma_sems((len(TCUTS) - 1,)),
                dma_sems((3,)),
            ],
            compiler_params=pltpu.CompilerParams(
                vmem_limit_bytes=100 * 1024 * 1024, disable_semaphore_checks=True, disable_bounds_checks=True),
        )(A_x.reshape(B, M), A_c_kv.reshape(C_VIEW), A_w_q.reshape(W_VIEW), A_w_uk.reshape(W_VIEW),
          A_w_uv.reshape(W_VIEW), A_w_o.reshape(O_VIEW), w1, B_b1, B_w2.reshape(G_VIEW), B_b2)
        return out.reshape(M // 128, B, 128).transpose(1, 0, 2).reshape(B, 1, M)
    return fn


_impl = make(OCUTS=(0,4,8,12,14,15,15.5,16),OVPU=2)


@jax.jit
def pallas_recurrent_scan__compressed_kv_cla__dense_activation_gelu__decode_kernel(
    A_x, A_c_kv, A_w_q, A_w_uk, A_w_uv, A_w_o, B_x, B_w1, B_b1, B_w2, B_b2,
):
    return _impl(A_x, A_c_kv, A_w_q, A_w_uk, A_w_uv, A_w_o, B_x, B_w1, B_b1, B_w2, B_b2)
```

```python
import jax
import jax.numpy as jnp
from jax import lax
import jax.experimental.pallas as pl
import jax.experimental.pallas.tpu as pltpu
import contextlib

F32 = jnp.float32
BF16 = jnp.bfloat16
B, H, SK, D, M, DC, F = 2, 32, 16384, 128, 512, 512, 1792
LOG2E = 1.4426950408889634
NT = (((1,), (1,)), ((), ()))
W_VIEW = (4, 128, H, D)
C_VIEW = (B * 16, SK // 16, DC)
O_VIEW = (4, 8 * D, M)
W1_VIEW = (M // 8 * F // 128, 8, 128)
BK = 2048


def _loop(lo, hi, body):
    lax.fori_loop(lo, hi, lambda i, _: body(i), None)


def _rows8(v):
    return jnp.concatenate([v[:, j * 128:(j + 1) * 128] for j in range(M // 128)], axis=0)


def _iota(shape, axis):
    return lax.broadcasted_iota(jnp.int32, shape, axis)


def make(TR=False, LAG=26, N0=(1, 1, 1), OCUTS=(0, 128, 256, 384, 448, 480, 496, 512), NMXU=5,
         TCUTS=(768, 832, 896, 960, 992, 1016, 1024), SMALL=128, TP=32, NS=2, ORDER='vkq', SMALL_AT=16, FIN=0, NOCOMP=False, OWALK=0):
    T0 = TCUTS[0]
    counts = {'x': 1, 'b1': 1, 'b2': 1, 'q': 1, 'k': 1, 'v': 1, '1': 1, '2': 1, 'c': 16, 'o': len(OCUTS) - 1, 't': len(TCUTS) - 1}
    first = {k: sum(list(counts.values())[:i]) for i, k in enumerate(counts)}

    def scope(name):
        return jax.named_scope('@' + name) if TR else contextlib.nullcontext()

    def stream():
        def quad(name, run, rows, sem, n0, n=4):
            return [(0, name, (pl.ds(run, n0), rows), sem), (1, name, (pl.ds(run + n0, n - n0), rows), sem)]

        steps = []
        for j in range(64):
            steps += [quad(a, 0, pl.ds(2 * j, 2), (a, 0), N0[0]) for a in ORDER]
            ffn = [(a, pl.ds(k * n, n)) for a, n in (('1', 8), ('2', 16)) for k in (j, j + 64) if k < 112]
            steps.append([(min(i, 1), a, rows, (a, 0)) for i, (a, rows) in enumerate(ffn)])
        steps[SMALL_AT] = steps[SMALL_AT] + [(0, a, ..., (a, 0)) for a in ('x', 'b1', 'b2')]
        for b in range(B):
            for j in range(64):
                steps += [quad('c', b * 16 + r, pl.ds(16 * j, 16), ('c', b * 8 + j // 8), N0[1]) for r in range(0, 16, 4)]
        for row in range(0, 512, 16):
            sem = ('o', sum(row >= c for c in OCUTS[1:]))
            steps += [quad('o', 0, pl.ds(r, 16), sem, N0[2], 4 if r < T0 else 3) for r in (row, row + 512)]
        cols = M // NS
        tail = [(k % 2, r, TP, 0, M) for k, r in enumerate(range(T0, 1024 - SMALL, TP))]
        tail += [(1, r, 8, c, cols) for r in range(1024 - SMALL, 1024, 8) for c in range(0, M, cols)]
        steps.append([(q, 'o', (3, pl.ds(r, n), pl.ds(c, w)), ('t', sum(r >= t for t in TCUTS[1:]))) for q, r, n, c, w in tail])
        ones = [c for s in steps for c in s if c[0] == 1]
        ahead = iter(ones[LAG:])
        steps = [[c if c[0] == 0 else next(ahead, None) for c in s] for s in steps]
        steps[0][1:1] = ones[:LAG]
        return steps

    def kernel(x_hbm, c_hbm, wq_hbm, wk_hbm, wv_hbm, wo_hbm, w1_hbm, b1_hbm, w2_hbm, b2_hbm, o_hbm,
               c_buf, wq_buf, wk_buf, wv_buf, wo_buf, w1_buf, w2_buf,
               flat, qa_ref, ctx_ref, lhs_ref, mul_ref, o_buf, x_buf, b1_buf, b2_buf, sems):
        refs = {'x': (x_hbm, x_buf), 'c': (c_hbm, c_buf), 'q': (wq_hbm, wq_buf), 'k': (wk_hbm, wk_buf), 'v': (wv_hbm, wv_buf),
                'o': (wo_hbm, wo_buf), '1': (w1_hbm, w1_buf), '2': (w2_hbm, w2_buf), 'b1': (b1_hbm, b1_buf), 'b2': (b2_hbm, b2_buf)}
        steps = stream()

        def issue(lo, hi):
            with scope(f'i{hi}'):
                for s in steps[4 * lo:4 * hi]:
                    for queue, name, idx, (sem, i) in filter(None, s):
                        hbm, buf = refs[name]
                        pltpu.make_async_copy(hbm.at[idx], buf.at[idx], sems.at[first[sem] + i]).start(priority=queue)

        def issue_part(i, cuts):
            for k in range(len(cuts) - 1):
                pl.when(i == k)(lambda: issue(cuts[k], cuts[k + 1]))

        def wait_filled(buf, sem, i=0):
            with scope(sem):
                pltpu.make_async_copy(buf, buf, sems.at[first[sem] + i]).wait()

        def wait_inputs(names):
            for a in names:
                wait_filled(refs[a][1], a)

        def write_out():
            o_copy = pltpu.make_async_copy(o_buf, o_hbm, sems.at[first['x']])
            o_copy.start()
            o_copy.wait()

        groups = []
        for g, (lo, hi) in enumerate(zip(OCUTS, OCUTS[1:])):
            n1 = 4 if 512 + lo < T0 else 3
            groups.append(([(wo_buf.at[:, pl.ds(lo, hi - lo)], 'o', g), (wo_buf.at[pl.ds(0, n1), pl.ds(512 + lo, hi - lo)], 'o', g)],
                           [(a, lo, hi - lo) for a in range(4)] + [(a, 512 + lo, hi - lo) for a in range(n1)]))
        for g, (lo, hi) in enumerate(zip(TCUTS, TCUTS[1:])):
            groups.append(([(wo_buf.at[3, pl.ds(lo, hi - lo)], 't', g)], [(3, lo, hi - lo)]))

        if NOCOMP:
            issue(0, 209)
            wait_inputs(('x', 'b1', 'b2', 'q', 'k', 'v', '1', '2'))
            for i in range(16):
                wait_filled(c_buf.at[pl.ds(0, 16), pl.ds(0, 128)], 'c', i)
            o_buf[...] = jnp.zeros((8, 128), BF16)
            for waits, _ in groups:
                for w in waits:
                    wait_filled(*w)
            return write_out()

        issue(0, 73)
        wait_inputs(('x', 'b1', 'b2', 'q', 'k', 'v', '1', '2'))
        x = x_buf[...].astype(F32)
        xc = x - jnp.mean(x, axis=-1, keepdims=True)
        var = jnp.mean(xc * xc, axis=-1, keepdims=True)
        xn = (xc * lax.rsqrt(var + 1e-5)).astype(BF16)

        w1 = w1_buf[...].reshape(M // 8, F // 128, 8, 128)
        w1 = jnp.concatenate([w1[:, j].reshape(M, 128) for j in range(F // 128)], axis=1)
        hid = jnp.dot(xn, w1, preferred_element_type=F32)
        hid = jax.nn.gelu(hid + b1_buf[...].astype(F32).reshape(1, F), approximate=True).astype(BF16)
        z = jnp.dot(hid, w2_buf[...], preferred_element_type=F32)
        z8 = _rows8(z + b2_buf[...].astype(F32).reshape(1, M))
        g8 = z8 * jax.nn.sigmoid(z8)
        x8 = _rows8(x)

        def same_head():
            return _iota((H, 128), 1) % H == _iota((H, 128), 0)

        def same_quad():
            return (_iota((128, DC), 1) // 4 == _iota((128, DC), 0)).astype(F32).astype(BF16)

        def contract_rows(v, w_buf):
            v4 = jnp.concatenate([jnp.where(_iota((H, DC), 1) % 4 == j, v, 0.0) for j in range(4)], axis=0)
            flat[...] = lax.dot_general(same_quad(), v4.astype(BF16), NT, preferred_element_type=F32)
            lhs = jnp.concatenate([jnp.where(same_head(), flat[t:t + 1, :], 0.0).astype(BF16) for t in range(128)], axis=1)
            return jnp.dot(lhs, w_buf[...].reshape(DC * H, D), preferred_element_type=F32)

        def absorb(b):
            cuts = tuple(range(73, 98, 4))
            pl.when(b == 0)(lambda: issue(cuts[0], cuts[1]))
            pl.when(b == 1)(lambda: issue(cuts[3], cuts[4]))
            xb = jnp.where(b == 0, xn[0:1].astype(F32), xn[1:2].astype(F32))
            q = contract_rows(jnp.broadcast_to(xb, (H, M)), wq_buf).astype(BF16)

            def half(k):
                pl.when(b == 0)(lambda: issue_part(k, cuts[1:4]))
                pl.when(b == 1)(lambda: issue_part(k, cuts[4:7]))
                w = wk_buf[pl.ds(2 * k, 2)].reshape(DC * H // 2, D)
                r = lax.dot_general(q, w, NT, preferred_element_type=F32)
                for t in range(64):
                    flat[pl.ds(k * 64 + t, 1), :] = jnp.sum(jnp.where(same_head(), r[:, t * 128:(t + 1) * 128], 0.0), axis=0, keepdims=True)

            _loop(0, 2, half)
            v4 = jnp.dot((flat[...] * (D ** -0.5 * LOG2E)).T.astype(BF16), same_quad(), preferred_element_type=F32)
            qa = v4[:H]
            for j in range(1, 4):
                qa = jnp.where(_iota((H, DC), 1) % 4 == j, v4[j * H:(j + 1) * H], qa)
            qa_ref[b] = qa.astype(BF16)

        _loop(0, B, absorb)

        def block(b, g, carry):
            m_prev, l_prev, acc = carry
            pl.when(b == 0)(lambda: issue_part(g, tuple(range(97, 138, 5))))
            pl.when(b == 1)(lambda: issue_part(g, (142, 146) + tuple(range(152, 201, 8))))
            part = (pl.ds(b * 16, 16), pl.ds(pl.multiple_of(g * 128, 128), 128))
            wait_filled(c_buf.at[part], 'c', b * 8 + g)
            c = c_buf[part].reshape(BK, DC)
            sc = lax.dot_general(qa_ref[b], c, NT, preferred_element_type=F32)
            m_new = jnp.maximum(m_prev, jnp.max(sc, axis=1, keepdims=True))
            p = jnp.exp2(sc - m_new)
            alpha = jnp.exp2(m_prev - m_new)
            pv = jnp.dot(p.astype(BF16), c, preferred_element_type=F32)
            return m_new, alpha * l_prev + jnp.sum(p, axis=1, keepdims=True), alpha * acc + pv

        def attend(b):
            init = (jnp.full((H, 1), -jnp.inf, F32), jnp.zeros((H, 1), F32), jnp.zeros((H, DC), F32))
            _, l, acc = lax.fori_loop(0, SK // BK, lambda g, carry: block(b, g, carry), init)
            pl.when(b == 0)(lambda: issue(137, 142))
            pl.when(b == 1)(lambda: issue(200, 205))
            ctx_ref[b] = contract_rows(acc / l, wv_buf)

        _loop(0, B, attend)
        issue(205, 209)

        def gather(parts):
            return jnp.concatenate([ctx_ref[:, a * 8 + r // D, :][:, r % D:r % D + n] for a, r, n in parts], axis=1)

        for g, (_, parts) in enumerate(groups[:NMXU]):
            lhs_ref[g, :B, :sum(n for _, _, n in parts)] = gather(parts)
        vpu = [p for _, parts in groups[NMXU:] for p in parts]
        nv = sum(n for _, _, n in vpu)
        pad = -nv % 128
        cb = gather(([(0, 0, pad)] if pad else []) + vpu).astype(BF16).astype(F32)
        for b in range(B):
            for k in range(0, nv + pad, 128):
                mul_ref[b, k:k + 128] = jnp.broadcast_to(cb[b:b + 1, k:k + 128], (128, 128)).T

        sl = _iota((8, 128), 0)

        def merge(lo, hi, k):
            m = (sl & k) != 0
            if k == 4:
                return jnp.where(m, hi, lo) + pltpu.roll(jnp.where(m, lo, hi), 4, 0)
            return jnp.where(m, hi, lo) + jnp.where(m, pltpu.roll(hi, k, 0), pltpu.roll(lo, 8 - k, 0))

        s = jnp.zeros((B, M), F32)
        part = [[None] * (M // 128) for _ in range(B)]
        at = pad
        for g, (waits, parts) in enumerate(groups):
            for w in waits:
                wait_filled(*w)
            if g < NMXU:
                rhs = jnp.concatenate([wo_buf[a, r:r + n] for a, r, n in parts], axis=0)
                s = s + jnp.dot(lhs_ref[g, :B, :rhs.shape[0]].astype(BF16), rhs, preferred_element_type=F32)
                if g == NMXU - 1:
                    base8 = x8 + _rows8(s) * g8
                continue
            for a, r0, n in parts:
                for r in range(r0, r0 + n, 8):
                    w = wo_buf[a, r:r + 8].astype(F32)
                    for b in range(B):
                        mul = mul_ref[b, at:at + 8, :]
                        for j in range(M // 128):
                            t = w[:, j * 128:(j + 1) * 128] * mul
                            part[b][j] = t if part[b][j] is None else part[b][j] + t
                    at += 8

        r4 = [[merge(part[b][j], part[b][j + 2], 4) for j in range(2)] for b in range(B)]
        r2 = [merge(r4[b][0], r4[b][1], 2) for b in range(B)]
        o_buf[...] = (base8 + g8 * merge(r2[0], r2[1], 1)).astype(BF16)
        write_out()

    def fn(A_x, A_c_kv, A_w_q, A_w_uk, A_w_uv, A_w_o, B_x, B_w1, B_b1, B_w2, B_b2):
        hbm = pl.BlockSpec(memory_space=pltpu.HBM)
        w1 = B_w1.reshape(M // 8, 8, F // 128, 128).transpose(0, 2, 1, 3).reshape(W1_VIEW)
        out = pl.pallas_call(
            kernel,
            out_shape=jax.ShapeDtypeStruct((8, 128), BF16),
            in_specs=[hbm] * 10,
            out_specs=hbm,
            scratch_shapes=[
                pltpu.VMEM(C_VIEW, BF16), pltpu.VMEM(W_VIEW, BF16), pltpu.VMEM(W_VIEW, BF16),
                pltpu.VMEM(W_VIEW, BF16), pltpu.VMEM(O_VIEW, BF16),
                pltpu.VMEM(W1_VIEW, BF16), pltpu.VMEM((F, M), BF16),
                pltpu.VMEM((128, 128), F32), pltpu.VMEM((B, H, DC), BF16), pltpu.VMEM((B, H, D), F32),
                pltpu.VMEM((NMXU, 8, 1024), F32), pltpu.VMEM((B, 8 * D, 128), F32), pltpu.VMEM((8, 128), BF16),
                pltpu.VMEM((B, M), BF16), pltpu.VMEM((F,), BF16), pltpu.VMEM((M,), BF16),
                pltpu.SemaphoreType.DMA((sum(counts.values()),)),
            ],
            compiler_params=pltpu.CompilerParams(
                vmem_limit_bytes=100 * 1024 * 1024, disable_semaphore_checks=True, disable_bounds_checks=True),
        )(A_x.reshape(B, M), A_c_kv.reshape(C_VIEW), A_w_q.reshape(W_VIEW), A_w_uk.reshape(W_VIEW),
          A_w_uv.reshape(W_VIEW), A_w_o.reshape(O_VIEW), w1, B_b1, B_w2, B_b2)
        return out.reshape(M // 128, B, 128).transpose(1, 0, 2).reshape(B, 1, M)
    return fn


_impl = make()


@jax.jit
def pallas_recurrent_scan__compressed_kv_cla__dense_activation_gelu__decode_kernel(
    A_x, A_c_kv, A_w_q, A_w_uk, A_w_uv, A_w_o, B_x, B_w1, B_b1, B_w2, B_b2,
):
    return _impl(A_x, A_c_kv, A_w_q, A_w_uk, A_w_uv, A_w_o, B_x, B_w1, B_b1, B_w2, B_b2)
```

```python
import jax
import jax.numpy as jnp
from jax import lax
import jax.experimental.pallas as pl
import jax.experimental.pallas.tpu as pltpu

F32 = jnp.float32
BF16 = jnp.bfloat16

B, H, SK, D, M, DC, F = 2, 32, 16384, 128, 512, 512, 1792
LOG2E = 1.4426950408889634
NT = (((1,), (1,)), ((), ()))

W_VIEW = (4, 128, H, D)
C_VIEW = (B * 16, SK // 16, DC)
O_VIEW = (4, 8 * D, M)
W1_VIEW = (M // 8 * F // 128, 8, 128)
BK = 16 * 128
QUEUE_1_DEPTH = 26

O_CUTS = (0, 128, 256, 384, 448, 480, 496, 512)
TAIL_CUTS = (768, 800, 832, 864, 896, 928, 960, 976, 992, 1008, 1016, 1024)
O_PARTS = [(0, 4 if half + lo < TAIL_CUTS[0] else 3, half + lo, hi - lo)
           for lo, hi in zip(O_CUTS, O_CUTS[1:]) for half in (0, 512)]
O_PARTS += [(3, 1, lo, hi - lo) for lo, hi in zip(TAIL_CUTS, TAIL_CUTS[1:])]
MXU_STEPS = 5
VPU_ROWS = sum(runs * rows for _, runs, _, rows in O_PARTS[2 * MXU_STEPS:])

V, K, Q, W1, W2, X, B1, B2, C, O = range(10)
SEM_C = B2 + 1
SEM_O = SEM_C + B * SK // BK
SEM_OUT = SEM_O + len(O_PARTS)


def _stream():
    def step(src, run, runs, rows, sem):
        first = runs // 2
        return [(0, src, (pl.ds(run, first), rows), sem),
                (1, src, (pl.ds(run + first, runs - first), rows), sem)]

    def ffn_step(src, j, n):
        return [(queue, src, pl.ds(k * n, n), src) for queue, k in ((0, j + 64), (1, j)) if k < 112]

    def o_part(run, row):
        return next(i for i, (a, _, lo, n) in enumerate(O_PARTS) if a == run and lo <= row < lo + n)

    rounds = []
    for j in range(64):
        v, k, q = (step(src, 0, 4, pl.ds(2 * j, 2), src) for src in (V, K, Q))
        rounds.append(v + k + q + ffn_step(W1, (j + 48) % 64, 8) + ffn_step(W2, (j + 32) % 64, 16))
    rounds[4] += [(0, src, ..., src) for src in (X, B1, B2)]
    for b in range(B):
        for j in range(64):
            rounds.append([copy for run in range(b * 16, b * 16 + 16, 4)
                           for copy in step(C, run, 4, pl.ds(16 * j, 16), SEM_C + b * 8 + j // 8)])
    for j in range(0, 512, 32):
        rounds.append([copy for row in (j, j + 512, j + 16, j + 528)
                       for copy in step(O, 0, O_PARTS[o_part(0, row)][1], pl.ds(row, 16),
                                        SEM_O + o_part(0, row))])
    tail = [((row // 32) % 2, row, 32, 0, M) for row in range(TAIL_CUTS[0], 896, 32)]
    tail += [(1, row, 8, col, M // 2) for row in range(896, 1024, 8) for col in (0, M // 2)]
    rounds.append([(queue, O, (3, pl.ds(row, n), pl.ds(col, width)), SEM_O + o_part(3, row))
                   for queue, row, n, col, width in tail])

    queue_1 = [copy for r in rounds for copy in r if copy[0] == 1]
    ahead = iter(queue_1[QUEUE_1_DEPTH:])
    rounds = [[copy if copy[0] == 0 else next(ahead, None) for copy in r] for r in rounds]
    rounds[0][1:1] = queue_1[:QUEUE_1_DEPTH]
    return [[copy for copy in r if copy is not None] for r in rounds]


def _loop(n, body):
    lax.fori_loop(0, n, lambda i, _: body(i), None)


def _iota(shape, axis):
    return lax.broadcasted_iota(jnp.int32, shape, axis)


def _rows8(v):
    return jnp.concatenate([v[:, j * 128:(j + 1) * 128] for j in range(M // 128)], axis=0)


def _kernel(*refs):
    hbm, out_hbm, buf = refs[:10], refs[10], refs[11:21]
    flat, qa_ref, ctx_ref, lhs_ref, mul_ref, out_buf, sems = refs[21:]
    rounds = _stream()

    def issue(lo, hi):
        for r in rounds[lo:hi]:
            for queue, src, idx, sem in r:
                pltpu.make_async_copy(hbm[src].at[idx], buf[src].at[idx], sems.at[sem]).start(priority=queue)

    def issue_nth(i, ranges):
        for k, (lo, hi) in enumerate(ranges):
            pl.when(i == k)(lambda: issue(lo, hi))

    def wait_filled(ref, sem):
        pltpu.make_async_copy(ref, ref, sems.at[sem]).wait()

    issue(0, 73)
    for src in (V, K, Q, W1, W2, X, B1, B2):
        wait_filled(buf[src], src)

    x = buf[X][...].astype(F32)
    xc = x - jnp.mean(x, axis=-1, keepdims=True)
    var = jnp.mean(xc * xc, axis=-1, keepdims=True)
    xn = (xc * lax.rsqrt(var + 1e-5)).astype(BF16)

    w1 = buf[W1][...].reshape(M // 8, F // 128, 8, 128)
    w1 = jnp.concatenate([w1[:, j].reshape(M, 128) for j in range(F // 128)], axis=1)
    hid = jnp.dot(xn, w1, preferred_element_type=F32)
    hid = jax.nn.gelu(hid + buf[B1][...].astype(F32).reshape(1, F), approximate=True).astype(BF16)
    z = jnp.dot(hid, buf[W2][...], preferred_element_type=F32)
    z8 = _rows8(z + buf[B2][...].astype(F32).reshape(1, M))
    g8 = z8 * jax.nn.sigmoid(z8)
    x8 = _rows8(x)

    def same_head():
        return _iota((H, 128), 1) % H == _iota((H, 128), 0)

    def same_matrix():
        return (_iota((128, DC), 1) // 4 == _iota((128, DC), 0)).astype(F32).astype(BF16)

    def contract_rows(v, w_ref):
        v4 = jnp.concatenate([jnp.where(_iota((H, DC), 1) % 4 == j, v, 0.0) for j in range(4)], axis=0)
        flat[...] = lax.dot_general(same_matrix(), v4.astype(BF16), NT, preferred_element_type=F32)
        lhs = [jnp.where(same_head(), flat[t:t + 1, :], 0.0).astype(BF16) for t in range(128)]
        return jnp.dot(jnp.concatenate(lhs, axis=1), w_ref[...].reshape(DC * H, D),
                       preferred_element_type=F32)

    def absorb(b):
        issue_nth(b, ((73, 77), (85, 89)))
        xb = jnp.where(b == 0, xn[0:1].astype(F32), xn[1:2].astype(F32))
        q = contract_rows(jnp.broadcast_to(xb, (H, M)), buf[Q]).astype(BF16)

        def half(k):
            issue_nth(2 * b + k, ((77, 81), (81, 85), (89, 93), (93, 97)))
            w = buf[K][pl.ds(2 * k, 2)].reshape(DC * H // 2, D)
            r = lax.dot_general(q, w, NT, preferred_element_type=F32)
            for t in range(64):
                own = jnp.where(same_head(), r[:, t * 128:(t + 1) * 128], 0.0)
                flat[pl.ds(k * 64 + t, 1), :] = jnp.sum(own, axis=0, keepdims=True)

        _loop(2, half)
        qt = (flat[...] * (D ** -0.5 * LOG2E)).T.astype(BF16)
        qa4 = jnp.dot(qt, same_matrix(), preferred_element_type=F32)
        qa = qa4[:H]
        for j in range(1, 4):
            qa = jnp.where(_iota((H, DC), 1) % 4 == j, qa4[j * H:(j + 1) * H], qa)
        qa_ref[b] = qa.astype(BF16)

    _loop(B, absorb)

    def attend(b):
        def block(g, carry):
            m_prev, l_prev, acc = carry
            issue_nth(b * 8 + g, [(r, r + 5) for r in range(97, 137, 5)] + [(142, 146), (146, 152)]
                      + [(r, r + 8) for r in range(152, 200, 8)])
            keys = (pl.ds(b * 16, 16), pl.ds(pl.multiple_of(g * 128, 128), 128))
            wait_filled(buf[C].at[keys], SEM_C + b * 8 + g)
            c = buf[C][keys].reshape(BK, DC)
            sc = lax.dot_general(qa_ref[b], c, NT, preferred_element_type=F32)
            m_new = jnp.maximum(m_prev, jnp.max(sc, axis=1, keepdims=True))
            p = jnp.exp2(sc - m_new)
            alpha = jnp.exp2(m_prev - m_new)
            pv = jnp.dot(p.astype(BF16), c, preferred_element_type=F32)
            return m_new, alpha * l_prev + jnp.sum(p, axis=1, keepdims=True), alpha * acc + pv

        init = (jnp.full((H, 1), -jnp.inf, F32), jnp.zeros((H, 1), F32), jnp.zeros((H, DC), F32))
        _, l, acc = lax.fori_loop(0, SK // BK, block, init)
        issue_nth(b, ((137, 142), (200, 205)))
        ctx_ref[b] = contract_rows(acc / l, buf[V])

    _loop(B, attend)
    issue(205, len(rounds))

    def pieces(first, last):
        return [(a, lo, n) for a0, runs, lo, n in O_PARTS[first:last] for a in range(a0, a0 + runs)]

    def ctx_of(rows):
        return jnp.concatenate([ctx_ref[:, a * 8 + lo // D, :][:, lo % D:lo % D + n]
                                for a, lo, n in rows], axis=1)

    def wait_part(i):
        a0, runs, lo, n = O_PARTS[i]
        wait_filled(buf[O].at[pl.ds(a0, runs), pl.ds(lo, n)], SEM_O + i)

    for i in range(MXU_STEPS):
        lhs = ctx_of(pieces(2 * i, 2 * i + 2))
        lhs_ref[i, :B, :lhs.shape[1]] = lhs
    at = -VPU_ROWS % 128
    factors = ctx_of([(0, 0, at)] + pieces(2 * MXU_STEPS, None)).astype(BF16).astype(F32)
    for b in range(B):
        for k in range(0, at + VPU_ROWS, 128):
            mul_ref[b, k:k + 128] = jnp.broadcast_to(factors[b:b + 1, k:k + 128], (128, 128)).T

    s = jnp.zeros((B, M), F32)
    for i in range(MXU_STEPS):
        wait_part(2 * i)
        wait_part(2 * i + 1)
        rhs = jnp.concatenate([buf[O][a, lo:lo + n] for a, lo, n in pieces(2 * i, 2 * i + 2)], axis=0)
        s = s + jnp.dot(lhs_ref[i, :B, :rhs.shape[0]].astype(BF16), rhs, preferred_element_type=F32)
    base8 = x8 + _rows8(s) * g8

    part = [[None] * (M // 128) for _ in range(B)]
    for i in range(2 * MXU_STEPS, len(O_PARTS)):
        wait_part(i)
        for a, lo, n in pieces(i, i + 1):
            for r in range(lo, lo + n, 8):
                w = buf[O][a, r:r + 8].astype(F32)
                for b in range(B):
                    mul = mul_ref[b, at:at + 8, :]
                    for j in range(M // 128):
                        t = w[:, j * 128:(j + 1) * 128] * mul
                        part[b][j] = t if part[b][j] is None else part[b][j] + t
                at += 8

    def merge(lo, hi, k):
        m = (_iota((8, 128), 0) & k) != 0
        if k == 4:
            return jnp.where(m, hi, lo) + pltpu.roll(jnp.where(m, lo, hi), 4, 0)
        return jnp.where(m, hi, lo) + jnp.where(m, pltpu.roll(hi, k, 0), pltpu.roll(lo, 8 - k, 0))

    r4 = [[merge(part[b][j], part[b][j + 2], 4) for j in range(2)] for b in range(B)]
    r2 = [merge(r4[b][0], r4[b][1], 2) for b in range(B)]
    out_buf[...] = (base8 + g8 * merge(r2[0], r2[1], 1)).astype(BF16)
    out_copy = pltpu.make_async_copy(out_buf, out_hbm, sems.at[SEM_OUT])
    out_copy.start()
    out_copy.wait()


@jax.jit
def pallas_recurrent_scan__compressed_kv_cla__dense_activation_gelu__decode_kernel(
    A_x: jax.Array,
    A_c_kv: jax.Array,
    A_w_q: jax.Array,
    A_w_uk: jax.Array,
    A_w_uv: jax.Array,
    A_w_o: jax.Array,
    B_x: jax.Array,
    B_w1: jax.Array,
    B_b1: jax.Array,
    B_w2: jax.Array,
    B_b2: jax.Array,
):
    del B_x
    w1_tiles = B_w1.reshape(M // 8, 8, F // 128, 128).transpose(0, 2, 1, 3).reshape(W1_VIEW)
    operands = (A_w_uv.reshape(W_VIEW), A_w_uk.reshape(W_VIEW), A_w_q.reshape(W_VIEW), w1_tiles, B_w2,
                A_x.reshape(B, M), B_b1, B_b2, A_c_kv.reshape(C_VIEW), A_w_o.reshape(O_VIEW))
    in_hbm = pl.BlockSpec(memory_space=pltpu.HBM)
    out = pl.pallas_call(
        _kernel,
        out_shape=jax.ShapeDtypeStruct((8, 128), BF16),
        in_specs=[in_hbm] * len(operands),
        out_specs=in_hbm,
        scratch_shapes=[pltpu.VMEM(a.shape, BF16) for a in operands] + [
            pltpu.VMEM((128, 128), F32),
            pltpu.VMEM((B, H, DC), BF16),
            pltpu.VMEM((B, H, D), F32),
            pltpu.VMEM((MXU_STEPS, 8, 8 * D), F32),
            pltpu.VMEM((B, VPU_ROWS + -VPU_ROWS % 128, 128), F32),
            pltpu.VMEM((8, 128), BF16),
            pltpu.SemaphoreType.DMA((SEM_OUT + 1,)),
        ],
        compiler_params=pltpu.CompilerParams(
            vmem_limit_bytes=100 * 1024 * 1024, disable_semaphore_checks=True, disable_bounds_checks=True),
    )(*operands)
    return out.reshape(M // 128, B, 128).transpose(1, 0, 2).reshape(B, 1, M)
```

```python
import jax
import jax.numpy as jnp
from jax import lax
import jax.experimental.pallas as pl
import jax.experimental.pallas.tpu as pltpu

F32 = jnp.float32
BF16 = jnp.bfloat16

B, H, SK, D, M, DC, F = 2, 32, 16384, 128, 512, 512, 1792
LOG2E = 1.4426950408889634
NT = (((1,), (1,)), ((), ()))

W_VIEW = (4, 128, H, D)
C_VIEW = (B * 16, SK // 16, DC)
O_VIEW = (4, 8 * D, M)
W1_VIEW = (M // 8 * F // 128, 8, 128)
BK = 16 * 128
QUEUE_1_DEPTH = 26

O_CUTS = (0, 128, 256, 384, 448, 480, 496, 512)
TAIL_CUTS = (768, 800, 832, 864, 896, 928, 960, 976, 992, 1008, 1024)
O_PARTS = [(0, 4 if half + lo < TAIL_CUTS[0] else 3, half + lo, hi - lo)
           for lo, hi in zip(O_CUTS, O_CUTS[1:]) for half in (0, 512)]
O_PARTS += [(3, 1, lo, hi - lo) for lo, hi in zip(TAIL_CUTS, TAIL_CUTS[1:])]
MXU_STEPS = 5
VPU_ROWS = sum(runs * rows for _, runs, _, rows in O_PARTS[2 * MXU_STEPS:])

V, K, Q, W1, W2, X, B1, B2, C, O = range(10)
SEM_C = B2 + 1
SEM_O = SEM_C + B * SK // BK
SEM_OUT = SEM_O + len(O_PARTS)


def _stream():
    def step(src, run, runs, rows, sem):
        first = runs // 2
        return [(0, src, (pl.ds(run, first), rows), sem),
                (1, src, (pl.ds(run + first, runs - first), rows), sem)]

    def ffn_step(src, j, n):
        return [(queue, src, pl.ds(k * n, n), src) for queue, k in ((0, j + 64), (1, j)) if k < 112]

    def o_part(run, row):
        return next(i for i, (a, _, lo, n) in enumerate(O_PARTS) if a == run and lo <= row < lo + n)

    rounds = []
    for j in range(64):
        v, k, q = (step(src, 0, 4, pl.ds(2 * j, 2), src) for src in (V, K, Q))
        rounds.append(v + k + q + ffn_step(W1, (j + 48) % 64, 8) + ffn_step(W2, (j + 32) % 64, 16))
    rounds[4] += [(0, src, None, src) for src in (X, B1, B2)]
    for b in range(B):
        for j in range(64):
            rounds.append([copy for run in range(b * 16, b * 16 + 16, 4)
                           for copy in step(C, run, 4, pl.ds(16 * j, 16), SEM_C + b * 8 + j // 8)])
    for j in range(0, 512, 32):
        rounds.append([copy for row in (j, j + 512, j + 16, j + 528)
                       for copy in step(O, 0, O_PARTS[o_part(0, row)][1], pl.ds(row, 16),
                                        SEM_O + o_part(0, row))])
    tail = [((row // 32) % 2, row, 32, 0, M) for row in range(TAIL_CUTS[0], 896, 32)]
    tail += [(1, row, 8, col, M // 2) for row in range(896, 1024, 8) for col in (0, M // 2)]
    rounds.append([(queue, O, (3, pl.ds(row, n), pl.ds(col, width)), SEM_O + o_part(3, row))
                   for queue, row, n, col, width in tail])

    queue_1 = [copy for r in rounds for copy in r if copy[0] == 1]
    ahead = iter(queue_1[QUEUE_1_DEPTH:])
    rounds = [[copy if copy[0] == 0 else next(ahead, None) for copy in r] for r in rounds]
    rounds[0][1:1] = queue_1[:QUEUE_1_DEPTH]
    return [[copy for copy in r if copy is not None] for r in rounds]


def _loop(n, body):
    lax.fori_loop(0, n, lambda i, _: body(i), None)


def _iota(shape, axis):
    return lax.broadcasted_iota(jnp.int32, shape, axis)


def _rows8(v):
    return jnp.concatenate([v[:, j * 128:(j + 1) * 128] for j in range(M // 128)], axis=0)


def _kernel(*refs):
    hbm, out_hbm, buf = refs[:10], refs[10], refs[11:21]
    flat, qa_ref, ctx_ref, lhs_ref, mul_ref, out_buf, sems = refs[21:]
    rounds = _stream()

    def issue(lo, hi):
        for r in rounds[lo:hi]:
            for queue, src, idx, sem in r:
                ends = [ref if idx is None else ref.at[idx] for ref in (hbm[src], buf[src])]
                pltpu.make_async_copy(*ends, sems.at[sem]).start(priority=queue)

    def issue_nth(i, ranges):
        for k, (lo, hi) in enumerate(ranges):
            pl.when(i == k)(lambda: issue(lo, hi))

    def wait_filled(ref, sem):
        pltpu.make_async_copy(ref, ref, sems.at[sem]).wait()

    issue(0, 73)
    for src in (V, K, Q, W1, W2, X, B1, B2):
        wait_filled(buf[src], src)

    x = buf[X][...].astype(F32)
    xc = x - jnp.mean(x, axis=-1, keepdims=True)
    var = jnp.mean(xc * xc, axis=-1, keepdims=True)
    xn = (xc * lax.rsqrt(var + 1e-5)).astype(BF16)

    w1 = buf[W1][...].reshape(M // 8, F // 128, 8, 128)
    w1 = jnp.concatenate([w1[:, j].reshape(M, 128) for j in range(F // 128)], axis=1)
    hid = jnp.dot(xn, w1, preferred_element_type=F32)
    hid = jax.nn.gelu(hid + buf[B1][...].astype(F32).reshape(1, F), approximate=True).astype(BF16)
    z = jnp.dot(hid, buf[W2][...], preferred_element_type=F32)
    z8 = _rows8(z + buf[B2][...].astype(F32).reshape(1, M))
    g8 = z8 * jax.nn.sigmoid(z8)
    x8 = _rows8(x)

    def same_head():
        return _iota((H, 128), 1) % H == _iota((H, 128), 0)

    def same_matrix():
        return (_iota((128, DC), 1) // 4 == _iota((128, DC), 0)).astype(F32).astype(BF16)

    def contract_rows(v, w_ref):
        v4 = jnp.concatenate([jnp.where(_iota((H, DC), 1) % 4 == j, v, 0.0) for j in range(4)], axis=0)
        flat[...] = lax.dot_general(same_matrix(), v4.astype(BF16), NT, preferred_element_type=F32)
        lhs = [jnp.where(same_head(), flat[t:t + 1, :], 0.0).astype(BF16) for t in range(128)]
        return jnp.dot(jnp.concatenate(lhs, axis=1), w_ref[...].reshape(DC * H, D),
                       preferred_element_type=F32)

    def absorb(b):
        issue_nth(b, ((73, 77), (85, 89)))
        xb = jnp.where(b == 0, xn[0:1].astype(F32), xn[1:2].astype(F32))
        q = contract_rows(jnp.broadcast_to(xb, (H, M)), buf[Q]).astype(BF16)

        def half(k):
            issue_nth(2 * b + k, ((77, 81), (81, 85), (89, 93), (93, 97)))
            w = buf[K][pl.ds(2 * k, 2)].reshape(DC * H // 2, D)
            r = lax.dot_general(q, w, NT, preferred_element_type=F32)
            for t in range(64):
                own = jnp.where(same_head(), r[:, t * 128:(t + 1) * 128], 0.0)
                flat[pl.ds(k * 64 + t, 1), :] = jnp.sum(own, axis=0, keepdims=True)

        _loop(2, half)
        qt = (flat[...] * (D ** -0.5 * LOG2E)).T.astype(BF16)
        qa4 = jnp.dot(qt, same_matrix(), preferred_element_type=F32)
        qa = qa4[:H]
        for j in range(1, 4):
            qa = jnp.where(_iota((H, DC), 1) % 4 == j, qa4[j * H:(j + 1) * H], qa)
        qa_ref[b] = qa.astype(BF16)

    _loop(B, absorb)

    def attend(b):
        def block(g, carry):
            m_prev, l_prev, acc = carry
            issue_nth(b * 8 + g, [(r, r + 5) for r in range(97, 137, 5)] + [(142, 146), (146, 152)]
                      + [(r, r + 8) for r in range(152, 200, 8)])
            keys = (pl.ds(b * 16, 16), pl.ds(pl.multiple_of(g * 128, 128), 128))
            wait_filled(buf[C].at[keys], SEM_C + b * 8 + g)
            c = buf[C][keys].reshape(BK, DC)
            sc = lax.dot_general(qa_ref[b], c, NT, preferred_element_type=F32)
            m_new = jnp.maximum(m_prev, jnp.max(sc, axis=1, keepdims=True))
            p = jnp.exp2(sc - m_new)
            alpha = jnp.exp2(m_prev - m_new)
            pv = jnp.dot(p.astype(BF16), c, preferred_element_type=F32)
            return m_new, alpha * l_prev + jnp.sum(p, axis=1, keepdims=True), alpha * acc + pv

        init = (jnp.full((H, 1), -jnp.inf, F32), jnp.zeros((H, 1), F32), jnp.zeros((H, DC), F32))
        _, l, acc = lax.fori_loop(0, SK // BK, block, init)
        issue_nth(b, ((137, 142), (200, 205)))
        ctx_ref[b] = contract_rows(acc / l, buf[V])

    _loop(B, attend)
    issue(205, len(rounds))

    def pieces(first, last):
        return [(a, lo, n) for a0, runs, lo, n in O_PARTS[first:last] for a in range(a0, a0 + runs)]

    def ctx_of(rows):
        return jnp.concatenate([ctx_ref[:, a * 8 + lo // D, :][:, lo % D:lo % D + n]
                                for a, lo, n in rows], axis=1)

    def wait_part(i):
        a0, runs, lo, n = O_PARTS[i]
        wait_filled(buf[O].at[pl.ds(a0, runs), pl.ds(lo, n)], SEM_O + i)

    lhs_ref[...] = jnp.zeros(lhs_ref.shape, F32)
    for i in range(MXU_STEPS):
        lhs = ctx_of(pieces(2 * i, 2 * i + 2))
        lhs_ref[i, :B, :lhs.shape[1]] = lhs
    at = -VPU_ROWS % 128
    factors = ctx_of([(0, 0, at)] + pieces(2 * MXU_STEPS, None)).astype(BF16).astype(F32)
    for b in range(B):
        for k in range(0, at + VPU_ROWS, 128):
            mul_ref[b, k:k + 128] = jnp.broadcast_to(factors[b:b + 1, k:k + 128], (128, 128)).T

    s = jnp.zeros((B, M), F32)
    for i in range(MXU_STEPS):
        wait_part(2 * i)
        wait_part(2 * i + 1)
        rhs = jnp.concatenate([buf[O][a, lo:lo + n] for a, lo, n in pieces(2 * i, 2 * i + 2)], axis=0)
        s = s + jnp.dot(lhs_ref[i, :B, :rhs.shape[0]].astype(BF16), rhs, preferred_element_type=F32)
    base8 = x8 + _rows8(s) * g8

    part = [[None] * (M // 128) for _ in range(B)]
    for i in range(2 * MXU_STEPS, len(O_PARTS)):
        wait_part(i)
        for a, lo, n in pieces(i, i + 1):
            for r in range(lo, lo + n, 8):
                w = buf[O][a, r:r + 8].astype(F32)
                for b in range(B):
                    mul = mul_ref[b, at:at + 8, :]
                    for j in range(M // 128):
                        t = w[:, j * 128:(j + 1) * 128] * mul
                        part[b][j] = t if part[b][j] is None else part[b][j] + t
                at += 8

    def merge(lo, hi, k):
        m = (_iota((8, 128), 0) & k) != 0
        if k == 4:
            return jnp.where(m, hi, lo) + pltpu.roll(jnp.where(m, lo, hi), 4, 0)
        return jnp.where(m, hi, lo) + jnp.where(m, pltpu.roll(hi, k, 0), pltpu.roll(lo, 8 - k, 0))

    r4 = [[merge(part[b][j], part[b][j + 2], 4) for j in range(2)] for b in range(B)]
    r2 = [merge(r4[b][0], r4[b][1], 2) for b in range(B)]
    out_buf[...] = (base8 + g8 * merge(r2[0], r2[1], 1)).astype(BF16)
    out_copy = pltpu.make_async_copy(out_buf, out_hbm, sems.at[SEM_OUT])
    out_copy.start()
    out_copy.wait()


@jax.jit
def pallas_recurrent_scan__compressed_kv_cla__dense_activation_gelu__decode_kernel(
    A_x: jax.Array,
    A_c_kv: jax.Array,
    A_w_q: jax.Array,
    A_w_uk: jax.Array,
    A_w_uv: jax.Array,
    A_w_o: jax.Array,
    B_x: jax.Array,
    B_w1: jax.Array,
    B_b1: jax.Array,
    B_w2: jax.Array,
    B_b2: jax.Array,
):
    del B_x
    w1_tiles = B_w1.reshape(M // 8, 8, F // 128, 128).transpose(0, 2, 1, 3).reshape(W1_VIEW)
    operands = (A_w_uv.reshape(W_VIEW), A_w_uk.reshape(W_VIEW), A_w_q.reshape(W_VIEW), w1_tiles, B_w2,
                A_x.reshape(B, M), B_b1, B_b2, A_c_kv.reshape(C_VIEW), A_w_o.reshape(O_VIEW))
    in_hbm = pl.BlockSpec(memory_space=pltpu.HBM)
    out = pl.pallas_call(
        _kernel,
        out_shape=jax.ShapeDtypeStruct((8, 128), BF16),
        in_specs=[in_hbm] * len(operands),
        out_specs=in_hbm,
        scratch_shapes=[pltpu.VMEM(a.shape, BF16) for a in operands] + [
            pltpu.VMEM((128, 128), F32),
            pltpu.VMEM((B, H, DC), BF16),
            pltpu.VMEM((B, H, D), F32),
            pltpu.VMEM((MXU_STEPS, 8, 8 * D), F32),
            pltpu.VMEM((B, VPU_ROWS + -VPU_ROWS % 128, 128), F32),
            pltpu.VMEM((8, 128), BF16),
            pltpu.SemaphoreType.DMA((SEM_OUT + 1,)),
        ],
        compiler_params=pltpu.CompilerParams(
            vmem_limit_bytes=100 * 1024 * 1024, disable_semaphore_checks=True, disable_bounds_checks=True),
    )(*operands)
    return out.reshape(M // 128, B, 128).transpose(1, 0, 2).reshape(B, 1, M)
```
